```python
import os as _os
_os.environ.setdefault("JAX_PLATFORMS", "cpu")
import jax
import jax.numpy as jnp

def _softmax(x, axis=-1):
    return jax.nn.softmax(x, axis=axis)
def _gelu(x):
    return jax.nn.gelu(x, approximate=True)
def _silu(x):
    return jax.nn.silu(x)
def _sigmoid(x):
    return jax.nn.sigmoid(x)
def _layernorm(x, axis=-1, eps=1e-5):
    m = jnp.mean(x, axis=axis, keepdims=True)
    v = jnp.var(x, axis=axis, keepdims=True)
    return (x - m) / jnp.sqrt(v + eps)
def _scatter_add(tgt, idx, src, axis=0):
    return tgt.at[idx].add(src)
def _segment_sum(src, seg, n):
    return jax.ops.segment_sum(src, seg, n)
class _Rng:
    def __init__(self, key):
        self._k = key
    def _next(self):
        self._k, sub = jax.random.split(self._k)
        return sub
    def normal(self, shape):
        return jax.random.normal(self._next(), shape, dtype=jnp.bfloat16)
    def randint(self, lo, hi, shape):
        return jax.random.randint(self._next(), shape, lo, hi, dtype=jnp.int32)
    def uniform(self, shape, lo=0.0, hi=1.0):
        return jax.random.uniform(self._next(), shape, jnp.bfloat16, lo, hi)
    def permutation(self, n):
        return jax.random.permutation(self._next(), n)


kernel_name = 'gated_mix__softmax_full_mha__dense_activation_relu__prompt'

def setup_inputs():
    _rng = _Rng(jax.random.key(int.from_bytes(__import__("os").urandom(4), "little")))
    _w = (lambda a: (lambda t: t.astype(jnp.bfloat16) if jnp.issubdtype(t.dtype, jnp.floating) else t)(jnp.asarray(a)))
    def _A_setup():
        B, S, D = 1, 2048, 640
        return {
            "x": _w((lambda *s: _rng.normal(s) * 0.05)(B, S, D)),
            "wqkv": _w((lambda *s: _rng.normal(s) * 0.8)(D, 3 * D)),
            "wo": _w((lambda *s: _rng.normal(s) * 0.05)(D, D)),
        }
    _A_in = _A_setup()

    def _B_setup():
        B, S, D, Dff = 1, 2048, 640, 1536
        return {
            "x": _w((lambda *s: _rng.normal(s) * 0.05)(B, S, D)),
            "w1": _w((lambda *s: _rng.normal(s) * 0.05)(D, Dff)),
            "w2": _w((lambda *s: _rng.normal(s) * 0.05)(Dff, D)),
        }
    _B_in = _B_setup()

    return {
        "A_x": _A_in["x"],
        "A_wqkv": _A_in["wqkv"],
        "A_wo": _A_in["wo"],
        "B_x": _B_in["x"],
        "B_w1": _B_in["w1"],
        "B_w2": _B_in["w2"],
        "gate_w": _w((lambda *s: _rng.normal(s) * 0.05)(640) * 16.0),
    }

def reference(A_x, A_wqkv, A_wo, B_x, B_w1, B_w2, gate_w):
    def _A_ref(x, wqkv, wo):
        B, S, D = x.shape
        H = 32; Dh = D // H
        qkv = (lambda x, *d: x.transpose(*d))((x @ wqkv).reshape(B, S, 3, H, Dh), 2, 0, 3, 1, 4)
        q, k, v = qkv[0], qkv[1], qkv[2]
        scale = Dh ** -0.5
        scores = jnp.einsum("bhqd,bhkd->bhqk", q, k) * scale
        p = _softmax(scores, axis=-1)
        o = jnp.einsum("bhqk,bhkd->bhqd", p, v)
        return (lambda x, *d: x.transpose(*d))(o, 0, 2, 1, 3).reshape(B, S, D) @ wo

    def _B_ref(x, w1, w2):
        h = jnp.einsum("bsd,df->bsf", x, w1)
        zero = jnp.zeros_like(h)
        h = jnp.maximum(h, zero)
        return jnp.einsum("bsf,fd->bsd", h, w2)

    x = A_x
    g = _sigmoid((x * gate_w).sum(-1, keepdims=True))
    a = _A_ref(x, A_wqkv, A_wo)
    b = _B_ref(x, B_w1, B_w2)
    return g * a + (1 - g) * b
```

```python
import functools, math
import jax, jax.numpy as jnp
from jax import lax
from jax.experimental import pallas as pl
from jax.experimental.pallas import tpu as pltpu

S, D, H, DH, DFF = 2048, 640, 32, 20, 1536
LOG2E = 1.4426950408889634
F32, BF16, U32 = jnp.float32, jnp.bfloat16, jnp.uint32

def head_window(h):
    lo = DH * h
    w = lo // 128
    if (lo + DH - 1) // 128 == w:
        return w, lo - 128 * w
    return 5 + w, lo - (128 * w + 64)

NT = (((1,), (1,)), ((), ()))
NN = (((1,), (0,)), ((), ()))

def make_kernel(TQS, CH, TK, HU, KU32, EXP):
    NC = S // CH
    NKC = S // TK
    NQS = S // TQS
    QPC = CH // TQS

    def kernel(x_hbm, wqkv_hbm, wo_hbm, w1_hbm, w2_hbm, gw_ref, out_hbm,
               x_v, wqkv_v, wo_v, w1_v, w2_v, out_v,
               kwin_scr, vt_scr, qb_scr, wqvt_scr, s_scr, m_scr, ot_scr, sems):
        def cp_x(c):
            return pltpu.make_async_copy(x_hbm.at[pl.ds(c * CH, CH), :], x_v.at[pl.ds(c * CH, CH), :], sems.at[c])
        def cp_w(j):
            return pltpu.make_async_copy(wqkv_hbm.at[:, pl.ds(j * D, D)], wqkv_v.at[j], sems.at[NC + j])
        cp_wo = pltpu.make_async_copy(wo_hbm, wo_v, sems.at[NC + 3])
        cp_w1 = pltpu.make_async_copy(w1_hbm, w1_v, sems.at[NC + 4])
        cp_w2 = pltpu.make_async_copy(w2_hbm, w2_v, sems.at[NC + 5])
        def cp_out(c):
            return pltpu.make_async_copy(out_v.at[pl.ds(c * CH, CH), :], out_hbm.at[pl.ds(c * CH, CH), :], sems.at[NC + 6 + c])

        cp_w(0).start(); cp_w(2).start(); cp_w(1).start(); cp_x(0).start(); cp_x(1).start()
        for c in range(2, NC):
            cp_x(c).start()

        def rows_of(c):
            return pl.ds(c * CH, CH) if isinstance(c, int) else pl.ds(pl.multiple_of(c * CH, CH), CH)

        def hrows(c):
            return pl.ds(c * (CH // 2), CH // 2) if isinstance(c, int) else pl.ds(pl.multiple_of(c * (CH // 2), CH // 2), CH // 2)

        def kstore(w, c, val):
            if KU32:
                kwin_scr[w, hrows(c), :] = pltpu.bitcast(val, U32)
            else:
                kwin_scr[w, c * CH:(c + 1) * CH, :] = val
        def kload(w, k0, n):
            if KU32:
                return pltpu.bitcast(kwin_scr[w, k0 // 2:(k0 + n) // 2, :], BF16)
            return kwin_scr[w, k0:k0 + n, :]

        def kproj(c):
            rows = rows_of(c)
            k = jnp.dot(x_v[rows, :], wqkv_v[1], preferred_element_type=F32)
            for w in range(5):
                kstore(w, c, k[:, 128 * w:128 * (w + 1)].astype(BF16))
            if not KU32:
                for w in range(4):
                    kstore(5 + w, c, k[:, 128 * w + 64:128 * (w + 1) + 64].astype(BF16))

        def kshift(c):
            if KU32:
                r = hrows(c)
                lane = lax.broadcasted_iota(jnp.int32, (CH // 2, 128), 1)
                rolled = [pltpu.roll(kwin_scr[w, r, :], 64, 1) for w in range(5)]
                for w in range(4):
                    kwin_scr[5 + w, r, :] = jnp.where(lane < 64, rolled[w], rolled[w + 1])

        def qvproj(c):
            xc = x_v[rows_of(c), :]
            qv = lax.dot_general(wqvt_scr[...], xc, NT, preferred_element_type=F32)
            row = lax.broadcasted_iota(jnp.int32, (4, CH), 0)
            tail = jnp.where(row == 0, 1.0, 0.0).astype(F32)
            for h in range(H):
                w, off = head_window(h)
                pre = off % 16
                post = 32 - DH - pre
                parts = []
                if pre:
                    parts.append(jnp.zeros((pre, CH), F32))
                parts.append(qv[DH * h:DH * (h + 1), :] * (DH ** -0.5 * LOG2E))
                if post:
                    parts.append(jnp.zeros((post, CH), F32))
                qb_scr[c, h] = pltpu.bitcast(jnp.concatenate(parts, axis=0).astype(BF16), U32)
            for h in range(H):
                blk = jnp.concatenate([qv[D + DH * h:D + DH * (h + 1), :].astype(BF16).astype(F32), tail], axis=0)
                vt_scr[c, h, 0:24, :] = blk

        with jax.named_scope("wait0"):
            cp_w(0).wait()
        with jax.named_scope("tr0"):
            wqvt_scr[0:D, :] = wqkv_v[0].astype(F32).T.astype(BF16)
        with jax.named_scope("wait1"):
            cp_w(2).wait()
        with jax.named_scope("tr1"):
            wqvt_scr[D:2 * D, :] = wqkv_v[2].astype(F32).T.astype(BF16)
        with jax.named_scope("wait2"):
            cp_w(1).wait()
        with jax.named_scope("proj_rest"):
            def body1(c, carry):
                cp_x(c).wait()
                kproj(c)
                qvproj(c)
                kshift(c)
                return carry
            lax.fori_loop(0, NC, body1, 0)
        cp_w1.start(); cp_w2.start(); cp_wo.start()

        def win_of(h):
            if isinstance(h, int):
                w, off = head_window(h)
                return w, off // 16
            lo = DH * h
            w0 = lo // 128
            straddle = ((lo + DH - 1) // 128) != w0
            off = lo - 128 * w0 - jnp.where(straddle, 64, 0)
            return jnp.where(straddle, 5 + w0, w0), off // 16

        def unit(b, h_pv, h_qk, wr, qc, qo):
            qsl = slice(qo, qo + TQS)
            if h_qk is not None:
                w, r0 = wr
                if EXP & 1: w = 3
                if EXP & 4: r0 = 2
                if EXP & 8: h_qk = 5
                band = qb_scr[qc, h_qk, :, qsl]
                lo, hi = band[0:8], band[8:16]
                z = jnp.zeros_like(lo)
                groups = []
                for r in range(8):
                    if isinstance(r0, int):
                        groups.append(lo if r == r0 else (hi if r == r0 + 1 else z))
                    else:
                        g = z if r == 0 else jnp.where(r0 == r - 1, hi, z)
                        if r < 7:
                            g = jnp.where(r0 == r, lo, g)
                        groups.append(g)
                qm = pltpu.bitcast(jnp.concatenate(groups, axis=0), BF16)
                m_new = None
            if h_pv is not None:
                m_cur = m_scr[b, qc, 0:1, qsl]
                acc = None
            for c in range(NKC):
                ksl = slice(c * TK, (c + 1) * TK)
                vc, vo = (c * TK) // CH, (c * TK) % CH
                if h_pv is not None:
                    p = jnp.exp2(s_scr[b, qc, qo // TQS, ksl, :] - m_cur)
                if h_qk is not None:
                    s = jnp.dot(kload(w, c * TK, TK), qm, preferred_element_type=F32)
                    s_scr[b, qc, qo // TQS, ksl, :] = s
                    mc = jnp.max(s.reshape(TK // 8, 8, TQS), axis=0)
                    m_new = mc if m_new is None else jnp.maximum(m_new, mc)
                if h_pv is not None:
                    d = lax.dot_general(vt_scr[vc, 7 if EXP & 2 else h_pv, 0:24, vo:vo + TK], p, NN, preferred_element_type=F32)
                    acc = d if acc is None else acc + d
            if h_qk is not None:
                m_scr[b, qc, :, qsl] = jnp.broadcast_to(jnp.max(m_new, axis=0, keepdims=True), (8, TQS))
            if h_pv is not None:
                ot_scr[qc, h_pv, :, qsl] = acc * (1.0 / acc[DH:DH + 1, :])

        def stage(b, h_pv, h_qk):
            wr = win_of(h_qk) if h_qk is not None else None
            for qs in range(NQS):
                unit(b, h_pv, h_qk, wr, (qs * TQS) // CH, (qs * TQS) % CH)

        with jax.named_scope("stage0"):
            for b in range(HU):
                stage(b, None, b)
        def body(j, carry):
            for b in range(HU):
                stage(b, HU * j + b, HU * (j + 1) + b)
            return carry
        with jax.named_scope("mainloop"):
            lax.fori_loop(0, H // HU - 1, body, 0)
        cp_w1.wait(); cp_w2.wait(); cp_wo.wait()

        gw = gw_ref[...].astype(F32)
        def final(c):
            rows = rows_of(c)
            hs = []
            for j in range(QPC):
                r0 = c * CH + j * TQS
                rj = pl.ds(r0, TQS) if isinstance(c, int) else pl.ds(pl.multiple_of(r0, TQS), TQS)
                hs.append(jnp.maximum(jnp.dot(x_v[rj, :], w1_v[...], preferred_element_type=F32), 0.0).astype(BF16))
                for b in range(HU):
                    unit(b, H - HU + b, None, None, c, j * TQS)
            hdn = jnp.concatenate(hs, axis=0)
            xq = x_v[rows, :]
            bb = jnp.dot(hdn, w2_v[...], preferred_element_type=F32)
            ot = jnp.concatenate([ot_scr[c, h, 0:DH, :] for h in range(H)], axis=0)
            o = ot.T.astype(BF16)
            a = jnp.dot(o, wo_v[...], preferred_element_type=F32)
            gl = jnp.sum(xq.astype(F32) * gw, axis=-1, keepdims=True)
            g = jax.nn.sigmoid(gl)
            out_v[rows, :] = (g * a + (1.0 - g) * bb).astype(BF16)
            cp_out(c).start()
        def body3(c, carry):
            final(c)
            return carry
        with jax.named_scope("final"):
            lax.fori_loop(0, NC, body3, 0)
        with jax.named_scope("waitout"):
            for c in range(NC):
                cp_out(c).wait()

    return kernel

def build(TQS=128, CH=512, TK=256, HU=1, KU32=True, EXP=0):
    kernel = make_kernel(TQS, CH, TK, HU, KU32, EXP)
    NC = S // CH
    @jax.jit
    def f(A_x, A_wqkv, A_wo, B_x, B_w1, B_w2, gate_w):
        x = A_x.reshape(S, D)
        gw = gate_w.reshape(1, D)
        anyspec = pl.BlockSpec(memory_space=pl.ANY)
        out = pl.pallas_call(
            kernel,
            in_specs=[anyspec] * 5 + [pl.BlockSpec(memory_space=pltpu.VMEM)],
            out_specs=anyspec,
            out_shape=jax.ShapeDtypeStruct((S, D), BF16),
            scratch_shapes=[
                pltpu.VMEM((S, D), BF16),
                pltpu.VMEM((3, D, D), BF16),
                pltpu.VMEM((D, D), BF16),
                pltpu.VMEM((D, DFF), BF16),
                pltpu.VMEM((DFF, D), BF16),
                pltpu.VMEM((S, D), BF16),
                pltpu.VMEM((9, S // 2, 128), U32) if KU32 else pltpu.VMEM((9, S, 128), BF16),
                pltpu.VMEM((NC, H, 32, CH), F32),
                pltpu.VMEM((NC, H, 16, CH), U32),
                pltpu.VMEM((2 * D, D), BF16),
                pltpu.VMEM((HU, NC, CH // TQS, S, TQS), F32),
                pltpu.VMEM((HU, NC, 8, CH), F32),
                pltpu.VMEM((NC, H, 24, CH), F32),
                pltpu.SemaphoreType.DMA((2 * NC + 6,)),
            ],
            compiler_params=pltpu.CompilerParams(vmem_limit_bytes=110 * 1024 * 1024),
        )(x, A_wqkv, A_wo, B_w1, B_w2, gw)
        return out.reshape(1, S, D)
    return f


_KERNEL_FN = build(TK=128)


@jax.jit
def pallas_gated_mix__softmax_full_mha__dense_activation_relu__prompt_kernel(
    A_x: jax.Array,
    A_wqkv: jax.Array,
    A_wo: jax.Array,
    B_x: jax.Array,
    B_w1: jax.Array,
    B_w2: jax.Array,
    gate_w: jax.Array,
):
    return _KERNEL_FN(A_x, A_wqkv, A_wo, B_x, B_w1, B_w2, gate_w)
```

```python
import jax
import jax.numpy as jnp
from jax import lax
from jax.experimental import pallas as pl
from jax.experimental.pallas import tpu as pltpu

S, D, H, DH, DFF = 2048, 640, 32, 20, 1536
LOG2E = 1.4426950408889634
F32, BF16, U32 = jnp.float32, jnp.bfloat16, jnp.uint32
TQ = 128
NQ = S // TQ
NT_ = S // 128

NT = (((1,), (1,)), ((), ()))
NN = (((1,), (0,)), ((), ()))


class _NoScope:
    def __enter__(self):
        return self

    def __exit__(self, *a):
        return False


def make_kernel(CH, NV, PROF, LAG, LEAD, LEAD2, T0, TEND, NACC, ROLL, TAB):
    NC = S // CH
    QPC = CH // TQ
    NG = NV // 8
    scope = jax.named_scope if PROF else (lambda name: _NoScope())

    def kernel(x_hbm, wqkv_hbm, wo_hbm, w1_hbm, w2_hbm, gw_ref, out_hbm,
               x_v, wqkv_v, wo_v, w1_v, w2_v, out_v,
               kh_scr, vt_scr, qb_scr, qf_scr, wqvt_scr, s_scr, sv_scr,
               mm_scr, ot_scr, tab_scr, zero_smem, sems):
        def cp_x(c):
            return pltpu.make_async_copy(x_hbm.at[pl.ds(c * CH, CH), :], x_v.at[pl.ds(c * CH, CH), :], sems.at[c])

        def cp_w(j):
            return pltpu.make_async_copy(wqkv_hbm.at[:, pl.ds(j * D, D)], wqkv_v.at[j], sems.at[NC + j])
        cp_wo = pltpu.make_async_copy(wo_hbm, wo_v, sems.at[NC + 3])
        cp_w1 = pltpu.make_async_copy(w1_hbm, w1_v, sems.at[NC + 4])
        cp_w2 = pltpu.make_async_copy(w2_hbm, w2_v, sems.at[NC + 5])

        def cp_out(c):
            return pltpu.make_async_copy(out_v.at[pl.ds(c * CH, CH), :], out_hbm.at[pl.ds(c * CH, CH), :], sems.at[NC + 6 + c])

        cp_w(0).start(); cp_w(2).start(); cp_w(1).start()
        for c in range(NC):
            cp_x(c).start()
        zero_smem[0] = 0

        def rows_of(c, n=CH):
            return pl.ds(c * n, n) if isinstance(c, int) else pl.ds(pl.multiple_of(c * n, n), n)

        def kload(h, k0, n):
            return pltpu.bitcast(kh_scr[h, k0 // 2:(k0 + n) // 2, :], BF16)

        def kproj(c):
            k = jnp.dot(x_v[rows_of(c), :], wqkv_v[1], preferred_element_type=F32)
            r = rows_of(c, CH // 2)
            kw = [pltpu.bitcast(k[:, 128 * w:128 * (w + 1)].astype(BF16), U32) for w in range(5)]
            lane = lax.broadcasted_iota(jnp.int32, (CH // 2, 128), 1)
            for h in range(H):
                w, off = (DH * h) // 128, (DH * h) % 128
                val = kw[w] if off == 0 else pltpu.roll(kw[w], 128 - off, 1)
                if off + DH > 128:
                    val = jnp.where(lane < 128 - off, val, pltpu.roll(kw[w + 1], 128 - off, 1))
                kh_scr[h, r, :] = val

        def qvproj(c):
            xc = x_v[rows_of(c), :]
            qv = lax.dot_general(wqvt_scr[...], xc, NT, preferred_element_type=F32)
            row = lax.broadcasted_iota(jnp.int32, (4, CH), 0)
            tail = jnp.where(row == 0, 1.0, 0.0).astype(F32)
            zpad = jnp.zeros((32 - DH, CH), F32)
            for h in range(H):
                band = jnp.concatenate([qv[DH * h:DH * (h + 1), :] * (DH ** -0.5 * LOG2E), zpad], axis=0).astype(BF16)
                qb_scr[c, h] = pltpu.bitcast(band, U32)
                if NV:
                    qf_scr[c, h] = band.astype(F32)[0:24, :]
            for h in range(H):
                vt_scr[c, h] = jnp.concatenate([qv[D + DH * h:D + DH * (h + 1), :].astype(BF16).astype(F32), tail], axis=0)

        with scope("wait0"):
            cp_w(0).wait()
        with scope("tr0"):
            wqvt_scr[0:D, :] = wqkv_v[0].astype(F32).T.astype(BF16)
        with scope("wait1"):
            cp_w(2).wait()
        with scope("tr1"):
            wqvt_scr[D:2 * D, :] = wqkv_v[2].astype(F32).T.astype(BF16)
        with scope("wait2"):
            cp_w(1).wait()
        with scope("proj"):
            def body1(c, carry):
                cp_x(c).wait()
                kproj(c)
                qvproj(c)
                return carry
            lax.fori_loop(0, NC, body1, 0)
        cp_w1.start(); cp_w2.start(); cp_wo.start()

        def vt_load(h, k0, n):
            return vt_scr[k0 // CH, h, :, k0 % CH:k0 % CH + n]

        def s_tile(par, j, i):
            k0, k1 = 128 * i, 128 * (i + 1)
            if k1 <= NV:
                return sv_scr[par, j, k0:k1, :]
            if k0 >= NV:
                return s_scr[j, k0 - NV:k1 - NV, :]
            return jnp.concatenate([sv_scr[par, j, k0:NV, :], s_scr[j, 0:k1 - NV, :]], axis=0)

        def m_final(par, j):
            m = mm_scr[j]
            if NV:
                m = jnp.maximum(m, jnp.max(sv_scr[par, j].reshape(NG, 8, TQ), axis=0))
            return jnp.max(m, axis=0, keepdims=True)

        def pv_tile(h, par, j, i, m_cur):
            p = jnp.exp2(s_tile(par, j, i) - m_cur)
            return p

        def finish(h, qc, qo, acc):
            ot_scr[qc, h, :, qo:qo + TQ] = acc * (1.0 / acc[DH:DH + 1, :])

        NSLOT = NT_ * NQ
        NVV = NG * NQ
        if NV:
            NB = NVV - TEND
            vslot = [T0 + (v * (NSLOT - T0)) // NB for v in range(NB)] + [NSLOT - 1] * TEND

        def stage(h_pv, h_qk):
            zz = zero_smem[0]
            never = zz > 0
            par_w = h_qk % 2
            par_r = 1 - par_w
            kb_cache = {}
            pending = {}
            mcs = {}

            def tok(t):
                while t >= 0 and t not in mcs:
                    t -= 1
                return mcs.get(t)

            def get_kb(g, t):
                if g not in kb_cache:
                    gp, half = g // 2, g % 2
                    kk = kload(h_qk, 16 * gp, 16).astype(F32)[8 * half:8 * half + 8]
                    if tok(t - LEAD) is not None:
                        kk = jnp.where(never, tok(t - LEAD), kk)
                    if ROLL:
                        kb_cache[g] = [jnp.broadcast_to((kk if d < ROLL else pltpu.roll(kk, 128 - (d // ROLL) * ROLL, 1))[:, d % ROLL:d % ROLL + 1], (8, TQ)) for d in range(DH)]
                    else:
                        kb_cache[g] = [jnp.broadcast_to(kk[:, d:d + 1], (8, TQ)) for d in range(DH)]
                    if TAB:
                        for d in range(DH):
                            tab_scr[g % 2, d] = kb_cache[g][d]
                        kb_cache[g] = [tab_scr[g % 2 + zz, d] for d in range(DH)]
                return kb_cache[g]

            def vpu_vreg(v, t):
                g, j = v // NQ, v % NQ
                kb = get_kb(g, t)
                if LEAD2 and tok(t - LEAD2) is not None:
                    kb = [jnp.where(never, tok(t - LEAD2), kb[a]) for a in range(NACC)] + kb[NACC:]
                qc, qo = (j * TQ) // CH, (j * TQ) % CH
                accs = [None] * NACC
                for d in range(DH):
                    pr = kb[d] * qf_scr[qc, h_qk, d:d + 1, qo:qo + TQ]
                    accs[d % NACC] = pr if accs[d % NACC] is None else accs[d % NACC] + pr
                sv = accs[0]
                for a in accs[1:]:
                    sv = sv + a
                sv_scr[par_w, j, 8 * g:8 * g + 8, :] = sv
                pending.setdefault(t + LAG, []).append(sv)

            v = 0
            carry_links = []
            for j in range(NQ):
                qc, qo = (j * TQ) // CH, (j * TQ) % CH
                band = qb_scr[qc, h_qk, :, qo:qo + TQ]
                groups = [band[0:8], band[8:16]]
                m_new = None
                acc = None
                if h_pv is not None:
                    m_cur = m_final(par_r, j)
                for i in range(NT_):
                    t = j * NT_ + i
                    k0, k1 = max(NV, 128 * i), 128 * (i + 1)
                    if h_pv is not None:
                        p = jnp.exp2(s_tile(par_r, j, i) - m_cur)
                    carry_links += pending.pop(t, [])
                    if k1 > k0:
                        n = k1 - k0
                        gl = list(groups)
                        for a, sv in enumerate(carry_links):
                            gl[1 - a % 2] = jnp.where(never, pltpu.bitcast(sv, U32), gl[1 - a % 2])
                        carry_links = []
                        qm = pltpu.bitcast(jnp.concatenate(gl, axis=0), BF16)
                        s = jnp.dot(kload(h_qk, k0, n)[:, 0:32], qm, preferred_element_type=F32)
                        s_scr[j, k0 - NV:k1 - NV, :] = s
                        mc = jnp.max(s.reshape(n // 8, 8, TQ), axis=0)
                        mcs[t] = mc
                        m_new = mc if m_new is None else jnp.maximum(m_new, mc)
                    if h_pv is not None:
                        d = lax.dot_general(vt_load(h_pv, 128 * i, 128), p, NN, preferred_element_type=F32)
                        acc = d if acc is None else acc + d
                    while NV and v < NVV and vslot[v] == t:
                        vpu_vreg(v, t)
                        v += 1
                mm_scr[j] = m_new
                if h_pv is not None:
                    finish(h_pv, qc, qo, acc)
            assert v == NVV

        with scope("stage0"):
            stage(None, 0)

        def body(h, carry):
            stage(h, h + 1)
            return carry
        with scope("mainloop"):
            lax.fori_loop(0, H - 1, body, 0)
        cp_w1.wait(); cp_w2.wait(); cp_wo.wait()

        gw = gw_ref[...].astype(F32)

        def final(c, carry):
            rows = rows_of(c)
            hs = []
            for jj in range(QPC):
                j = c * QPC + jj
                hs.append(jnp.maximum(jnp.dot(x_v[rows_of(j, TQ), :], w1_v[...], preferred_element_type=F32), 0.0).astype(BF16))
                m_cur = m_final((H - 1) % 2, j)
                acc = None
                for i in range(NT_):
                    p = jnp.exp2(s_tile((H - 1) % 2, j, i) - m_cur)
                    d = lax.dot_general(vt_load(H - 1, 128 * i, 128), p, NN, preferred_element_type=F32)
                    acc = d if acc is None else acc + d
                finish(H - 1, c, jj * TQ, acc)
            hdn = jnp.concatenate(hs, axis=0)
            xq = x_v[rows, :]
            bb = jnp.dot(hdn, w2_v[...], preferred_element_type=F32)
            ot = jnp.concatenate([ot_scr[c, h, 0:DH, :] for h in range(H)], axis=0)
            o = ot.T.astype(BF16)
            a = jnp.dot(o, wo_v[...], preferred_element_type=F32)
            gl = jnp.sum(xq.astype(F32) * gw, axis=-1, keepdims=True)
            g = jax.nn.sigmoid(gl)
            out_v[rows, :] = (g * a + (1.0 - g) * bb).astype(BF16)
            cp_out(c).start()
            return carry
        with scope("final"):
            lax.fori_loop(0, NC, final, 0)
        with scope("waitout"):
            for c in range(NC):
                cp_out(c).wait()

    return kernel


def build(CH=512, NV=128, PROF=False, LAG=4, LEAD=24, LEAD2=12, T0=8, TEND=0, NACC=2, ROLL=2, TAB=0):
    kernel = make_kernel(CH, NV, PROF, LAG, LEAD, LEAD2, T0, TEND, NACC, ROLL, TAB)
    NC = S // CH

    @jax.jit
    def f(A_x, A_wqkv, A_wo, B_x, B_w1, B_w2, gate_w):
        x = A_x.reshape(S, D)
        gw = gate_w.reshape(1, D)
        anyspec = pl.BlockSpec(memory_space=pl.ANY)
        out = pl.pallas_call(
            kernel,
            in_specs=[anyspec] * 5 + [pl.BlockSpec(memory_space=pltpu.VMEM)],
            out_specs=anyspec,
            out_shape=jax.ShapeDtypeStruct((S, D), BF16),
            scratch_shapes=[
                pltpu.VMEM((S, D), BF16),
                pltpu.VMEM((3, D, D), BF16),
                pltpu.VMEM((D, D), BF16),
                pltpu.VMEM((D, DFF), BF16),
                pltpu.VMEM((DFF, D), BF16),
                pltpu.VMEM((S, D), BF16),
                pltpu.VMEM((H, S // 2, 128), U32),
                pltpu.VMEM((NC, H, 24, CH), F32),
                pltpu.VMEM((NC, H, 16, CH), U32),
                pltpu.VMEM((NC, H, 24, CH), F32),
                pltpu.VMEM((2 * D, D), BF16),
                pltpu.VMEM((NQ, S - NV, TQ), F32),
                pltpu.VMEM((2, NQ, max(NV, 8), TQ), F32),
                pltpu.VMEM((NQ, 8, TQ), F32),
                pltpu.VMEM((NC, H, 24, CH), F32),
                pltpu.VMEM((2, DH, 8, TQ), F32),
                pltpu.SMEM((1,), jnp.int32),
                pltpu.SemaphoreType.DMA((2 * NC + 6,)),
            ],
            compiler_params=pltpu.CompilerParams(vmem_limit_bytes=110 * 1024 * 1024),
        )(x, A_wqkv, A_wo, B_w1, B_w2, gw)
        return out.reshape(1, S, D)
    return f


_KERNEL_FN = build(NV=160,ROLL=2)


@jax.jit
def pallas_gated_mix__softmax_full_mha__dense_activation_relu__prompt_kernel(
    A_x: jax.Array,
    A_wqkv: jax.Array,
    A_wo: jax.Array,
    B_x: jax.Array,
    B_w1: jax.Array,
    B_w2: jax.Array,
    gate_w: jax.Array,
):
    return _KERNEL_FN(A_x, A_wqkv, A_wo, B_x, B_w1, B_w2, gate_w)
```

```python
import jax
import jax.numpy as jnp
from jax import lax
from jax.experimental import pallas as pl
from jax.experimental.pallas import tpu as pltpu

S, D, H, DH, DFF = 2048, 640, 32, 20, 1536
LOG2E = 1.4426950408889634
F32, BF16, U32 = jnp.float32, jnp.bfloat16, jnp.uint32
TQ = 128
NQ = S // TQ
NKT = S // 128
CH = 512
NC = S // CH
QPC = CH // TQ

NT = (((1,), (1,)), ((), ()))
NN = (((1,), (0,)), ((), ()))


class _NoScope:
    def __enter__(self):
        return self

    def __exit__(self, *a):
        return False


def make_kernel(NV, PROF, PM, P0, OSPLIT):
    NG = NV // 8
    scope = jax.named_scope if PROF else (lambda name: _NoScope())
    NO = NC * OSPLIT
    OR = S // NO

    def kernel(x_hbm, wqkv_hbm, wo_hbm, w1_hbm, w2_hbm, gw_hbm, out_hbm,
               x_v, wqkv_v, wo_v, w1_v, w2_v, out_v,
               kw_scr, kh_scr, vt_scr, qb_scr, qf_scr, wt_scr, s_scr, sv_scr,
               mm_scr, ot_scr, gw_ref, zero_smem, sems):
        def rows_of(c, n=CH):
            return pl.ds(c * n, n) if isinstance(c, int) else pl.ds(pl.multiple_of(c * n, n), n)

        def cp_x(c):
            return pltpu.make_async_copy(x_hbm.at[rows_of(c), :], x_v.at[rows_of(c), :], sems.at[c])

        def cp_w(j):
            return pltpu.make_async_copy(wqkv_hbm.at[:, pl.ds(j * D, D)], wqkv_v.at[j], sems.at[NC + j])
        cp_wo = pltpu.make_async_copy(wo_hbm, wo_v, sems.at[NC + 3])
        cp_w1 = pltpu.make_async_copy(w1_hbm, w1_v, sems.at[NC + 4])
        cp_w2 = pltpu.make_async_copy(w2_hbm, w2_v, sems.at[NC + 5])

        cp_gw = pltpu.make_async_copy(gw_hbm, gw_ref, sems.at[NC + 6 + NO])

        def cp_out(i):
            return pltpu.make_async_copy(out_v.at[rows_of(i, OR), :], out_hbm.at[rows_of(i, OR), :], sems.at[NC + 6 + i])

        cp_w(1).start(); cp_x(0).start(); cp_x(1).start(); cp_w(0).start()
        cp_x(2).start(); cp_w(2).start(); cp_x(3).start()
        zero_smem[0] = 0

        def kload(h, k0, n):
            return pltpu.bitcast(kh_scr[h, k0 // 2:(k0 + n) // 2, :], BF16)

        def kmat(c):
            k = jnp.dot(x_v[rows_of(c), :], wqkv_v[1], preferred_element_type=F32)
            for w in range(5):
                kw_scr[w, rows_of(c, CH // 2), :] = pltpu.bitcast(k[:, 128 * w:128 * (w + 1)].astype(BF16), U32)

        def krolls(c):
            r = rows_of(c, CH // 2)
            kw = [kw_scr[w, r, :] for w in range(5)]
            lane = lax.broadcasted_iota(jnp.int32, (CH // 2, 128), 1)
            for h in range(H):
                w, off = (DH * h) // 128, (DH * h) % 128
                val = kw[w] if off == 0 else pltpu.roll(kw[w], 128 - off, 1)
                if off + DH > 128:
                    val = jnp.where(lane < 128 - off, val, pltpu.roll(kw[w + 1], 128 - off, 1))
                kh_scr[h, r, :] = val

        def qvproj(c):
            xc = x_v[rows_of(c), :]
            qv = lax.dot_general(wt_scr[0:2 * D, :], xc, NT, preferred_element_type=F32)
            row = lax.broadcasted_iota(jnp.int32, (4, CH), 0)
            tail = jnp.where(row == 0, 1.0, 0.0).astype(F32)
            zpad = jnp.zeros((32 - DH, CH), F32)
            for h in range(H):
                band = jnp.concatenate([qv[DH * h:DH * (h + 1), :] * (DH ** -0.5 * LOG2E), zpad], axis=0).astype(BF16)
                qb_scr[c, h] = pltpu.bitcast(band, U32)
                qf_scr[c, h] = band.astype(F32)[0:24, :]
            for h in range(H):
                vt_scr[c, h] = jnp.concatenate([qv[D + DH * h:D + DH * (h + 1), :].astype(BF16).astype(F32), tail], axis=0)

        with scope("wait0"):
            cp_w(1).wait()
        with scope("projk"):
            def body0(c, carry):
                cp_x(c).wait()

                @pl.when(c == 1)
                def _():
                    cp_w(0).wait()

                @pl.when(c == 2)
                def _():
                    cp_w(2).wait()
                src = jnp.where(c == 0, 1, jnp.where(c == 1, 0, 2))
                dst = jnp.where(c == 0, 2, jnp.where(c == 1, 0, 1))
                kmat(c)
                wt_scr[rows_of(dst, D), :] = wqkv_v[src].astype(F32).T.astype(BF16)
                return carry
            lax.fori_loop(0, NC, body0, 0)
        cp_w1.start(); cp_w2.start(); cp_wo.start(); cp_gw.start()
        with scope("proj"):
            def body1(c, carry):
                qvproj(c)
                krolls(c)
                return carry
            lax.fori_loop(0, NC, body1, 0)

        def vt_load(h, i):
            k0 = 128 * i
            return vt_scr[k0 // CH, h, :, k0 % CH:k0 % CH + 128]

        def s_tile(par, j, i):
            k0, k1 = 128 * i, 128 * (i + 1)
            if k1 <= NV:
                return sv_scr[par, j, k0:k1, :]
            if k0 >= NV:
                return s_scr[j, k0 - NV:k1 - NV, :]
            return jnp.concatenate([sv_scr[par, j, k0:NV, :], s_scr[j, 0:k1 - NV, :]], axis=0)

        def m_final(par, j):
            m = jnp.maximum(mm_scr[j], jnp.max(sv_scr[par, j].reshape(NG, 8, TQ), axis=0))
            return jnp.max(m, axis=0, keepdims=True)

        def finish(h, qc, qo, acc):
            ot_scr[qc, h, :, qo:qo + TQ] = acc * (1.0 / acc[DH:DH + 1, :])

        NSLOT = NKT * NQ
        NVV = NG * NQ
        n16 = (S - NV) // 16
        sizes = sorted(16 * (((n16 * (u + 1)) // NKT) - ((n16 * u) // NKT)) for u in range(NKT))

        def stage(h_pv, h_qk, prm):
            LAG, LEAD, LEAD2, T0, NACC, ROLL, TOKM = prm
            vslot = [T0 + (v * (NSLOT - T0)) // NVV for v in range(NVV)]
            never = zero_smem[0] > 0
            par_w = h_qk % 2
            par_r = 1 - par_w
            kb_cache = {}
            pending = {}
            toks = {}

            def tok(t):
                while t >= 0 and t not in toks:
                    t -= 1
                return toks.get(t)

            def get_kb(g, t):
                if g not in kb_cache:
                    gp, half = g // 2, g % 2
                    kk = kload(h_qk, 16 * gp, 16).astype(F32)[8 * half:8 * half + 8]
                    if tok(t - LEAD) is not None:
                        kk = jnp.where(never, tok(t - LEAD), kk)
                    kb_cache[g] = [
                        jnp.broadcast_to(
                            (kk if d < ROLL else pltpu.roll(kk, 128 - (d // ROLL) * ROLL, 1))[:, d % ROLL:d % ROLL + 1],
                            (8, TQ))
                        for d in range(DH)]
                return kb_cache[g]

            def vpu_vreg(v, t):
                g, j = v // NQ, v % NQ
                kb = get_kb(g, t)
                if LEAD2 and tok(t - LEAD2) is not None:
                    kb = [jnp.where(never, tok(t - LEAD2), kb[a]) for a in range(NACC)] + kb[NACC:]
                qc, qo = (j * TQ) // CH, (j * TQ) % CH
                accs = [None] * NACC
                for d in range(DH):
                    pr = kb[d] * qf_scr[qc, h_qk, d:d + 1, qo:qo + TQ]
                    accs[d % NACC] = pr if accs[d % NACC] is None else accs[d % NACC] + pr
                sv = accs[0]
                for a in accs[1:]:
                    sv = sv + a
                sv_scr[par_w, j, 8 * g:8 * g + 8, :] = sv
                pending.setdefault(t + LAG, []).append(sv)

            v = 0
            for j in range(NQ):
                qc, qo = (j * TQ) // CH, (j * TQ) % CH
                band = qb_scr[qc, h_qk, :, qo:qo + TQ]
                groups = [band[0:8], band[8:16]]
                m_new = None
                acc = None
                ps = {}
                if h_pv is not None:
                    m_cur = m_final(par_r, j)
                k0 = NV
                for u in range(NKT):
                    t = j * NKT + u
                    n = sizes[u]
                    if h_pv is not None:
                        for i in range(max(u + 1, (k0 + n + 127) // 128)):
                            if i not in ps:
                                ps[i] = jnp.exp2(s_tile(par_r, j, i) - m_cur)
                    gl = list(groups)
                    for a, sv in enumerate(pending.pop(t, [])):
                        gl[1 - a % 2] = jnp.where(never, pltpu.bitcast(sv, U32), gl[1 - a % 2])
                    qm = pltpu.bitcast(jnp.concatenate(gl, axis=0), BF16)
                    s = jnp.dot(kload(h_qk, k0, n)[:, 0:32], qm, preferred_element_type=F32)
                    s_scr[j, k0 - NV:k0 + n - NV, :] = s
                    mc = jnp.max(s.reshape(n // 8, 8, TQ), axis=0)
                    m_new = mc if m_new is None else jnp.maximum(m_new, mc)
                    toks[t] = m_new if TOKM else mc
                    k0 += n
                    if h_pv is not None:
                        d = lax.dot_general(vt_load(h_pv, u), ps[u], NN, preferred_element_type=F32)
                        acc = d if acc is None else acc + d
                        toks[t] = acc[0:8]
                    while v < NVV and vslot[v] <= t:
                        vpu_vreg(v, t)
                        v += 1
                assert k0 == S
                mm_scr[j] = m_new
                if h_pv is not None:
                    finish(h_pv, qc, qo, acc)
            assert v == NVV

        with scope("stage0"):
            stage(None, 0, P0)

        def body(h, carry):
            stage(h, h + 1, PM)
            return carry
        with scope("mainloop"):
            lax.fori_loop(0, H - 1, body, 0)
        cp_w1.wait(); cp_w2.wait(); cp_wo.wait(); cp_gw.wait()

        gw = gw_ref[...].astype(F32).reshape(1, D)

        def final(c, carry):
            hs = []
            for jj in range(QPC):
                j = c * QPC + jj
                hs.append(jnp.maximum(jnp.dot(x_v[rows_of(j, TQ), :], w1_v[...], preferred_element_type=F32), 0.0).astype(BF16))
                m_cur = m_final((H - 1) % 2, j)
                acc = None
                for i in range(NKT):
                    p = jnp.exp2(s_tile((H - 1) % 2, j, i) - m_cur)
                    d = lax.dot_general(vt_load(H - 1, i), p, NN, preferred_element_type=F32)
                    acc = d if acc is None else acc + d
                finish(H - 1, c, jj * TQ, acc)
            hdn = jnp.concatenate(hs, axis=0)
            bb = jnp.dot(hdn, w2_v[...], preferred_element_type=F32)
            ot = jnp.concatenate([ot_scr[c, h, 0:DH, :] for h in range(H)], axis=0)
            o = ot.T.astype(BF16)
            for q in range(OSPLIT):
                i = c * OSPLIT + q
                a = jnp.dot(o[q * OR:(q + 1) * OR, :], wo_v[...], preferred_element_type=F32)
                xq = x_v[rows_of(i, OR), :]
                gl = jnp.sum(xq.astype(F32) * gw, axis=-1, keepdims=True)
                g = jax.nn.sigmoid(gl)
                out_v[rows_of(i, OR), :] = (g * a + (1.0 - g) * bb[q * OR:(q + 1) * OR, :]).astype(BF16)
                cp_out(i).start()
            return carry
        with scope("final"):
            lax.fori_loop(0, NC, final, 0)
        with scope("waitout"):
            for i in range(NO):
                cp_out(i).wait()

    return kernel


def build(NV=192, PROF=False, PM=(4, 22, 10, 12, 2, 2, 1), P0=(3, 20, 12, 8, 2, 4, 0), OSPLIT=2):
    kernel = make_kernel(NV, PROF, PM, P0, OSPLIT)

    @jax.jit
    def f(A_x, A_wqkv, A_wo, B_x, B_w1, B_w2, gate_w):
        x = A_x.reshape(S, D)
        gw = gate_w
        anyspec = pl.BlockSpec(memory_space=pl.ANY)
        out = pl.pallas_call(
            kernel,
            in_specs=[anyspec] * 6,
            out_specs=anyspec,
            out_shape=jax.ShapeDtypeStruct((S, D), BF16),
            scratch_shapes=[
                pltpu.VMEM((S, D), BF16),
                pltpu.VMEM((3, D, D), BF16),
                pltpu.VMEM((D, D), BF16),
                pltpu.VMEM((D, DFF), BF16),
                pltpu.VMEM((DFF, D), BF16),
                pltpu.VMEM((S, D), BF16),
                pltpu.VMEM((5, S // 2, 128), U32),
                pltpu.VMEM((H, S // 2, 128), U32),
                pltpu.VMEM((NC, H, 24, CH), F32),
                pltpu.VMEM((NC, H, 16, CH), U32),
                pltpu.VMEM((NC, H, 24, CH), F32),
                pltpu.VMEM((3 * D, D), BF16),
                pltpu.VMEM((NQ, S - NV, TQ), F32),
                pltpu.VMEM((2, NQ, NV, TQ), F32),
                pltpu.VMEM((NQ, 8, TQ), F32),
                pltpu.VMEM((NC, H, 24, CH), F32),
                pltpu.VMEM((D,), BF16),
                pltpu.SMEM((1,), jnp.int32),
                pltpu.SemaphoreType.DMA((NC + 7 + NC * OSPLIT,)),
            ],
            compiler_params=pltpu.CompilerParams(vmem_limit_bytes=110 * 1024 * 1024),
        )(x, A_wqkv, A_wo, B_w1, B_w2, gw)
        return out.reshape(1, S, D)
    return f


_KERNEL_FN = build()


@jax.jit
def pallas_gated_mix__softmax_full_mha__dense_activation_relu__prompt_kernel(
    A_x: jax.Array,
    A_wqkv: jax.Array,
    A_wo: jax.Array,
    B_x: jax.Array,
    B_w1: jax.Array,
    B_w2: jax.Array,
    gate_w: jax.Array,
):
    return _KERNEL_FN(A_x, A_wqkv, A_wo, B_x, B_w1, B_w2, gate_w)
```

```python
import jax
import jax.numpy as jnp
from jax import lax
from jax.experimental import pallas as pl
from jax.experimental.pallas import tpu as pltpu

S, D, H, DH, DFF = 2048, 640, 32, 20, 1536
LOG2E = 1.4426950408889634
F32, BF16, U32 = jnp.float32, jnp.bfloat16, jnp.uint32
TQ = 128
NQ = S // TQ
NKT = S // 128
CH = 512
NC = S // CH
QPC = CH // TQ
NV = 192
NG = NV // 8
OSPLIT = 2
NO = NC * OSPLIT
OR = S // NO

P_MAIN = (4, 16, 9, 16, 2, 2, 1, 3, 1)
P_FIRST = (4, 18, 7, 6, 2, 2, 1, 0, 1)

NT = (((1,), (1,)), ((), ()))
NN = (((1,), (0,)), ((), ()))


def _kernel(x_hbm, wqkv_hbm, wo_hbm, w1_hbm, w2_hbm, gw_hbm, out_hbm,
            x_v, wqkv_v, wo_v, w1_v, w2_v, out_v,
            kw_scr, kh_scr, vt_scr, qb_scr, qf_scr, wt_scr, s_scr, sv_scr,
            mm_scr, ot_scr, gw_ref, zero_smem, sems):
    def rows_of(c, n=CH):
        return pl.ds(c * n, n) if isinstance(c, int) else pl.ds(pl.multiple_of(c * n, n), n)

    def cp_x(c):
        return pltpu.make_async_copy(x_hbm.at[rows_of(c), :], x_v.at[rows_of(c), :], sems.at[c])

    def cp_w(j):
        return pltpu.make_async_copy(wqkv_hbm.at[:, pl.ds(j * D, D)], wqkv_v.at[j], sems.at[NC + j])

    cp_wo = pltpu.make_async_copy(wo_hbm, wo_v, sems.at[NC + 3])
    cp_w1 = pltpu.make_async_copy(w1_hbm, w1_v, sems.at[NC + 4])
    cp_w2 = pltpu.make_async_copy(w2_hbm, w2_v, sems.at[NC + 5])
    cp_gw = pltpu.make_async_copy(gw_hbm, gw_ref, sems.at[NC + 6 + NO])

    def cp_out(i):
        return pltpu.make_async_copy(out_v.at[rows_of(i, OR), :], out_hbm.at[rows_of(i, OR), :],
                                     sems.at[NC + 6 + i])

    cp_w(1).start(); cp_x(0).start(); cp_x(1).start(); cp_w(0).start()
    cp_x(2).start(); cp_w(2).start(); cp_x(3).start()
    zero_smem[0] = 0

    def kload(h, k0, n):
        return pltpu.bitcast(kh_scr[h, k0 // 2:(k0 + n) // 2, :], BF16)

    def kmat(c):
        k = jnp.dot(x_v[rows_of(c), :], wqkv_v[1], preferred_element_type=F32)
        for w in range(5):
            kw_scr[w, rows_of(c, CH // 2), :] = pltpu.bitcast(k[:, 128 * w:128 * (w + 1)].astype(BF16), U32)

    def krolls(c):
        r = rows_of(c, CH // 2)
        kw = [kw_scr[w, r, :] for w in range(5)]
        lane = lax.broadcasted_iota(jnp.int32, (CH // 2, 128), 1)
        for h in range(H):
            w, off = (DH * h) // 128, (DH * h) % 128
            val = kw[w] if off == 0 else pltpu.roll(kw[w], 128 - off, 1)
            if off + DH > 128:
                val = jnp.where(lane < 128 - off, val, pltpu.roll(kw[w + 1], 128 - off, 1))
            kh_scr[h, r, :] = val

    def qvproj(c):
        xc = x_v[rows_of(c), :]
        qv = lax.dot_general(wt_scr[0:2 * D, :], xc, NT, preferred_element_type=F32)
        row = lax.broadcasted_iota(jnp.int32, (4, CH), 0)
        tail = jnp.where(row == 0, 1.0, 0.0).astype(F32)
        zpad = jnp.zeros((32 - DH, CH), F32)
        for h in range(H):
            band = jnp.concatenate([qv[DH * h:DH * (h + 1), :] * (DH ** -0.5 * LOG2E), zpad], axis=0).astype(BF16)
            qb_scr[c, h] = pltpu.bitcast(band, U32)
            qf_scr[c, h] = band.astype(F32)[0:24, :]
        for h in range(H):
            vt_scr[c, h] = jnp.concatenate(
                [qv[D + DH * h:D + DH * (h + 1), :].astype(BF16).astype(F32), tail], axis=0)

    cp_w(1).wait()

    def body0(c, carry):
        cp_x(c).wait()

        @pl.when(c == 1)
        def _():
            cp_w(0).wait()

        @pl.when(c == 2)
        def _():
            cp_w(2).wait()
        src = jnp.where(c == 0, 1, jnp.where(c == 1, 0, 2))
        dst = jnp.where(c == 0, 2, jnp.where(c == 1, 0, 1))
        kmat(c)
        wt_scr[rows_of(dst, D), :] = wqkv_v[src].astype(F32).T.astype(BF16)
        return carry
    lax.fori_loop(0, NC, body0, 0)
    cp_w1.start(); cp_w2.start(); cp_wo.start(); cp_gw.start()

    def body1(c, carry):
        qvproj(c)
        krolls(c)
        return carry
    lax.fori_loop(0, NC, body1, 0)

    def vt_load(h, i):
        k0 = 128 * i
        return vt_scr[k0 // CH, h, :, k0 % CH:k0 % CH + 128]

    def s_tile(par, j, i):
        k0, k1 = 128 * i, 128 * (i + 1)
        if k1 <= NV:
            return sv_scr[par, j, k0:k1, :]
        if k0 >= NV:
            return s_scr[j, k0 - NV:k1 - NV, :]
        return jnp.concatenate([sv_scr[par, j, k0:NV, :], s_scr[j, 0:k1 - NV, :]], axis=0)

    def m_final(par, j):
        m = jnp.maximum(mm_scr[j], jnp.max(sv_scr[par, j].reshape(NG, 8, TQ), axis=0))
        return jnp.max(m, axis=0, keepdims=True)

    NSLOT = NKT * NQ
    NVV = NG * NQ
    n16 = (S - NV) // 16
    sizes = sorted(16 * (((n16 * (u + 1)) // NKT) - ((n16 * u) // NKT)) for u in range(NKT))

    def stage(h_pv, h_qk, prm):
        LAG, LEAD, LEAD2, T0, NACC, ROLL, TOKM, PVLAG, NGATE = prm
        vslot = [min(NSLOT - 1, T0 + (v * (NSLOT - T0)) // NVV) for v in range(NVV)]
        never = zero_smem[0] > 0
        par_w = h_qk % 2
        par_r = 1 - par_w
        kb_cache = {}
        pending = {}
        toks = {}

        def tok(t):
            while t >= 0 and t not in toks:
                t -= 1
            return toks.get(t)

        def get_kb(g, t):
            if g not in kb_cache:
                gp, half = g // 2, g % 2
                kk = kload(h_qk, 16 * gp, 16).astype(F32)[8 * half:8 * half + 8]
                if tok(t - LEAD) is not None:
                    kk = jnp.where(never, tok(t - LEAD), kk)
                kb_cache[g] = [
                    jnp.broadcast_to(
                        (kk if d < ROLL else pltpu.roll(kk, 128 - (d // ROLL) * ROLL, 1))[:, d % ROLL:d % ROLL + 1],
                        (8, TQ))
                    for d in range(DH)]
            return kb_cache[g]

        def vpu_vreg(v, t):
            g, j = v // NQ, v % NQ
            kb = get_kb(g, t)
            if tok(t - LEAD2) is not None:
                kb = [jnp.where(never, tok(t - LEAD2), kb[a]) for a in range(NGATE)] + kb[NGATE:]
            qc, qo = (j * TQ) // CH, (j * TQ) % CH
            accs = [None] * NACC
            for d in range(DH):
                pr = kb[d] * qf_scr[qc, h_qk, d:d + 1, qo:qo + TQ]
                accs[d % NACC] = pr if accs[d % NACC] is None else accs[d % NACC] + pr
            sv = accs[0]
            for a in accs[1:]:
                sv = sv + a
            sv_scr[par_w, j, 8 * g:8 * g + 8, :] = sv
            pending.setdefault(t + LAG, []).append(sv)

        v = 0
        ps = {}
        accs_pv = {}

        def do_pv(tp, t):
            jp, ip = tp // NKT, tp % NKT
            d = lax.dot_general(vt_load(h_pv, ip), ps.pop((jp, ip)), NN, preferred_element_type=F32)
            accs_pv[jp] = d if ip == 0 else accs_pv[jp] + d
            toks[t] = accs_pv[jp][0:8]
            if ip == NKT - 1:
                qo = (jp * TQ) % CH
                ot_scr[(jp * TQ) // CH, h_pv, :, qo:qo + TQ] = accs_pv.pop(jp)

        for j in range(NQ):
            qc, qo = (j * TQ) // CH, (j * TQ) % CH
            band = qb_scr[qc, h_qk, :, qo:qo + TQ]
            groups = [band[0:8], band[8:16]]
            m_new = None
            nps = 0
            if h_pv is not None:
                m_cur = m_final(par_r, j)
            k0 = NV
            for u in range(NKT):
                t = j * NKT + u
                n = sizes[u]
                if h_pv is not None:
                    while nps < max(u + 1, (k0 + n + 127) // 128):
                        ps[(j, nps)] = jnp.exp2(s_tile(par_r, j, nps) - m_cur)
                        nps += 1
                gl = list(groups)
                for a, sv in enumerate(pending.pop(t, [])):
                    gl[1 - a % 2] = jnp.where(never, pltpu.bitcast(sv, U32), gl[1 - a % 2])
                qm = pltpu.bitcast(jnp.concatenate(gl, axis=0), BF16)
                s = jnp.dot(kload(h_qk, k0, n)[:, 0:32], qm, preferred_element_type=F32)
                s_scr[j, k0 - NV:k0 + n - NV, :] = s
                mc = jnp.max(s.reshape(n // 8, 8, TQ), axis=0)
                m_new = mc if m_new is None else jnp.maximum(m_new, mc)
                toks[t] = m_new if TOKM else mc
                k0 += n
                if h_pv is not None and t >= PVLAG:
                    do_pv(t - PVLAG, t)
                while v < NVV and vslot[v] <= t:
                    vpu_vreg(v, t)
                    v += 1
            assert k0 == S
            mm_scr[j] = m_new
        if h_pv is not None:
            for tp in range(NSLOT - PVLAG, NSLOT):
                do_pv(tp, NSLOT - 1)
        assert v == NVV

    stage(None, 0, P_FIRST)

    def body(h, carry):
        stage(h, h + 1, P_MAIN)
        return carry
    lax.fori_loop(0, H - 1, body, 0)
    cp_w1.wait(); cp_w2.wait(); cp_wo.wait(); cp_gw.wait()

    gw = gw_ref[...].astype(F32).reshape(1, D)

    def final(c, carry):
        hs = []
        for jj in range(QPC):
            j = c * QPC + jj
            hs.append(jnp.maximum(
                jnp.dot(x_v[rows_of(j, TQ), :], w1_v[...], preferred_element_type=F32), 0.0).astype(BF16))
            m_cur = m_final((H - 1) % 2, j)
            acc = None
            for i in range(NKT):
                p = jnp.exp2(s_tile((H - 1) % 2, j, i) - m_cur)
                d = lax.dot_general(vt_load(H - 1, i), p, NN, preferred_element_type=F32)
                acc = d if acc is None else acc + d
            ot_scr[c, H - 1, :, jj * TQ:(jj + 1) * TQ] = acc
        hdn = jnp.concatenate(hs, axis=0)
        bb = jnp.dot(hdn, w2_v[...], preferred_element_type=F32)
        ot = jnp.concatenate(
            [ot_scr[c, h, 0:DH, :] * (1.0 / ot_scr[c, h, DH:DH + 1, :]) for h in range(H)], axis=0)
        o = ot.T.astype(BF16)
        for q in range(OSPLIT):
            i = c * OSPLIT + q
            a = jnp.dot(o[q * OR:(q + 1) * OR, :], wo_v[...], preferred_element_type=F32)
            xq = x_v[rows_of(i, OR), :]
            gl = jnp.sum(xq.astype(F32) * gw, axis=-1, keepdims=True)
            g = jax.nn.sigmoid(gl)
            out_v[rows_of(i, OR), :] = (g * a + (1.0 - g) * bb[q * OR:(q + 1) * OR, :]).astype(BF16)
            cp_out(i).start()
        return carry
    lax.fori_loop(0, NC, final, 0)
    for i in range(NO):
        cp_out(i).wait()


@jax.jit
def pallas_gated_mix__softmax_full_mha__dense_activation_relu__prompt_kernel(
    A_x: jax.Array,
    A_wqkv: jax.Array,
    A_wo: jax.Array,
    B_x: jax.Array,
    B_w1: jax.Array,
    B_w2: jax.Array,
    gate_w: jax.Array,
):
    del B_x
    anyspec = pl.BlockSpec(memory_space=pl.ANY)
    out = pl.pallas_call(
        _kernel,
        in_specs=[anyspec] * 6,
        out_specs=anyspec,
        out_shape=jax.ShapeDtypeStruct((S, D), BF16),
        scratch_shapes=[
            pltpu.VMEM((S, D), BF16),
            pltpu.VMEM((3, D, D), BF16),
            pltpu.VMEM((D, D), BF16),
            pltpu.VMEM((D, DFF), BF16),
            pltpu.VMEM((DFF, D), BF16),
            pltpu.VMEM((S, D), BF16),
            pltpu.VMEM((5, S // 2, 128), U32),
            pltpu.VMEM((H, S // 2, 128), U32),
            pltpu.VMEM((NC, H, 24, CH), F32),
            pltpu.VMEM((NC, H, 16, CH), U32),
            pltpu.VMEM((NC, H, 24, CH), F32),
            pltpu.VMEM((3 * D, D), BF16),
            pltpu.VMEM((NQ, S - NV, TQ), F32),
            pltpu.VMEM((2, NQ, NV, TQ), F32),
            pltpu.VMEM((NQ, 8, TQ), F32),
            pltpu.VMEM((NC, H, 24, CH), F32),
            pltpu.VMEM((D,), BF16),
            pltpu.SMEM((1,), jnp.int32),
            pltpu.SemaphoreType.DMA((NC + 7 + NO,)),
        ],
        compiler_params=pltpu.CompilerParams(vmem_limit_bytes=110 * 1024 * 1024),
    )(A_x.reshape(S, D), A_wqkv, A_wo, B_w1, B_w2, gate_w)
    return out.reshape(1, S, D)
```

```python
import jax
import jax.numpy as jnp
from jax import lax
from jax.experimental import pallas as pl
from jax.experimental.pallas import tpu as pltpu

S, D, H, DH, DFF = 2048, 640, 32, 20, 1536
LOG2E = 1.4426950408889634
F32, BF16, U32 = jnp.float32, jnp.bfloat16, jnp.uint32
TQ = 128
NQ = S // TQ
NKT = S // 128
CH = 512
NC = S // CH
QPC = CH // TQ
NV = 192
NG = NV // 8
OSPLIT = 2
NO = NC * OSPLIT
OR = S // NO
KSPL = 256

P_MAIN = (4, 16, 9, 16, 2, 2, 1, 3, 1)
P_FIRST = (4, 18, 7, 6, 2, 2, 1, 0, 1)

NT = (((1,), (1,)), ((), ()))
NN = (((1,), (0,)), ((), ()))


def _kernel(x_hbm, wqkv_hbm, wo_hbm, w1_hbm, w2_hbm, gw_hbm, out_hbm,
            x_v, wqkv_v, wo_v, w1_v, w2_v, out_v,
            kw_scr, kh_scr, vt_scr, qb_scr, qf_scr, wt_scr, s_scr, sv_scr,
            mm_scr, ot_scr, gw_ref, zero_smem, sems):
    def rows_of(c, n=CH):
        return pl.ds(c * n, n) if isinstance(c, int) else pl.ds(pl.multiple_of(c * n, n), n)

    def cp_x(c):
        return pltpu.make_async_copy(x_hbm.at[rows_of(c), :], x_v.at[rows_of(c), :], sems.at[c])

    def cp_w(j):
        return pltpu.make_async_copy(wqkv_hbm.at[:, pl.ds(j * D, D)], wqkv_v.at[j], sems.at[NC + j])

    def cp_wk(part):
        c0, c1 = (0, KSPL) if part == 0 else (KSPL, D)
        return pltpu.make_async_copy(wqkv_hbm.at[:, pl.ds(D + c0, c1 - c0)], wqkv_v.at[1, :, pl.ds(c0, c1 - c0)],
                                     sems.at[NC + 1] if part == 0 else sems.at[NC + 7 + NO])

    def cp_x0(part):
        r = pl.ds(part * (CH // 2), CH // 2)
        return pltpu.make_async_copy(x_hbm.at[r, :], x_v.at[r, :],
                                     sems.at[0] if part == 0 else sems.at[NC + 8 + NO])

    cp_wo = pltpu.make_async_copy(wo_hbm, wo_v, sems.at[NC + 3])
    cp_w1 = pltpu.make_async_copy(w1_hbm, w1_v, sems.at[NC + 4])
    cp_w2 = pltpu.make_async_copy(w2_hbm, w2_v, sems.at[NC + 5])
    cp_gw = pltpu.make_async_copy(gw_hbm, gw_ref, sems.at[NC + 6 + NO])

    def cp_out(i):
        return pltpu.make_async_copy(out_v.at[rows_of(i, OR), :], out_hbm.at[rows_of(i, OR), :],
                                     sems.at[NC + 6 + i])

    cp_wk(0).start(); cp_x0(0).start(); cp_x0(1).start(); cp_wk(1).start()
    cp_x(1).start(); cp_x(2).start(); cp_w(0).start()
    cp_x(3).start(); cp_w(2).start()
    zero_smem[0] = 0

    def kload(h, k0, n):
        return pltpu.bitcast(kh_scr[h, k0 // 2:(k0 + n) // 2, :], BF16)

    def kmat(c):
        k = jnp.dot(x_v[rows_of(c), :], wqkv_v[1], preferred_element_type=F32)
        for w in range(5):
            kw_scr[w, rows_of(c, CH // 2), :] = pltpu.bitcast(k[:, 128 * w:128 * (w + 1)].astype(BF16), U32)

    def krolls(c):
        r = rows_of(c, CH // 2)
        kw = [kw_scr[w, r, :] for w in range(5)]
        lane = lax.broadcasted_iota(jnp.int32, (CH // 2, 128), 1)
        for h in range(H):
            w, off = (DH * h) // 128, (DH * h) % 128
            val = kw[w] if off == 0 else pltpu.roll(kw[w], 128 - off, 1)
            if off + DH > 128:
                val = jnp.where(lane < 128 - off, val, pltpu.roll(kw[w + 1], 128 - off, 1))
            kh_scr[h, r, :] = val

    def qvproj(c):
        xc = x_v[rows_of(c), :]
        qv = lax.dot_general(wt_scr[0:2 * D, :], xc, NT, preferred_element_type=F32)
        row = lax.broadcasted_iota(jnp.int32, (4, CH), 0)
        tail = jnp.where(row == 0, 1.0, 0.0).astype(F32)
        zpad = jnp.zeros((32 - DH, CH), F32)
        for h in range(H):
            band = jnp.concatenate([qv[DH * h:DH * (h + 1), :] * (DH ** -0.5 * LOG2E), zpad], axis=0).astype(BF16)
            qb_scr[c, h] = pltpu.bitcast(band, U32)
            qf_scr[c, h] = band.astype(F32)[0:24, :]
        for h in range(H):
            vt_scr[c, h] = jnp.concatenate(
                [qv[D + DH * h:D + DH * (h + 1), :].astype(BF16).astype(F32), tail], axis=0)

    def kmat0(c0, c1, m0, m1):
        for mh in range(m0, m1):
            r0 = mh * TQ
            k = jnp.dot(x_v[r0:r0 + TQ, :], wqkv_v[1, :, c0:c1], preferred_element_type=F32)
            for w in range(c0 // 128, c1 // 128):
                kw_scr[w, r0 // 2:(r0 + TQ) // 2, :] = pltpu.bitcast(
                    k[:, 128 * w - c0:128 * (w + 1) - c0].astype(BF16), U32)

    cp_wk(0).wait(); cp_x0(0).wait()
    kmat0(0, KSPL, 0, QPC // 2)
    cp_x0(1).wait()
    kmat0(0, KSPL, QPC // 2, QPC)
    cp_wk(1).wait()
    kmat0(KSPL, D, 0, QPC)

    def body0(c, carry):
        cp_x(c).wait()

        @pl.when(c == 2)
        def _():
            cp_w(0).wait()

        @pl.when(c == 3)
        def _():
            cp_w(2).wait()
        src = jnp.where(c == 1, 1, jnp.where(c == 2, 0, 2))
        dst = jnp.where(c == 1, 2, jnp.where(c == 2, 0, 1))
        kmat(c)
        wt_scr[rows_of(dst, D), :] = wqkv_v[src].astype(F32).T.astype(BF16)
        return carry
    lax.fori_loop(1, NC, body0, 0)
    cp_w1.start(); cp_w2.start(); cp_wo.start(); cp_gw.start()

    def body1(c, carry):
        qvproj(c)
        krolls(c)
        return carry
    lax.fori_loop(0, NC, body1, 0)

    def vt_load(h, i):
        k0 = 128 * i
        return vt_scr[k0 // CH, h, :, k0 % CH:k0 % CH + 128]

    def s_tile(par, j, i):
        k0, k1 = 128 * i, 128 * (i + 1)
        if k1 <= NV:
            return sv_scr[par, j, k0:k1, :]
        if k0 >= NV:
            return s_scr[j, k0 - NV:k1 - NV, :]
        return jnp.concatenate([sv_scr[par, j, k0:NV, :], s_scr[j, 0:k1 - NV, :]], axis=0)

    def m_final(par, j):
        m = jnp.maximum(mm_scr[j], jnp.max(sv_scr[par, j].reshape(NG, 8, TQ), axis=0))
        return jnp.max(m, axis=0, keepdims=True)

    NSLOT = NKT * NQ
    NVV = NG * NQ
    n16 = (S - NV) // 16
    sizes = sorted(16 * (((n16 * (u + 1)) // NKT) - ((n16 * u) // NKT)) for u in range(NKT))

    def stage(h_pv, h_qk, prm):
        LAG, LEAD, LEAD2, T0, NACC, ROLL, TOKM, PVLAG, NGATE = prm
        vslot = [min(NSLOT - 1, T0 + (v * (NSLOT - T0)) // NVV) for v in range(NVV)]
        never = zero_smem[0] > 0
        par_w = h_qk % 2
        par_r = 1 - par_w
        kb_cache = {}
        pending = {}
        toks = {}

        def tok(t):
            while t >= 0 and t not in toks:
                t -= 1
            return toks.get(t)

        def get_kb(g, t):
            if g not in kb_cache:
                gp, half = g // 2, g % 2
                kk = kload(h_qk, 16 * gp, 16).astype(F32)[8 * half:8 * half + 8]
                if tok(t - LEAD) is not None:
                    kk = jnp.where(never, tok(t - LEAD), kk)
                kb_cache[g] = [
                    jnp.broadcast_to(
                        (kk if d < ROLL else pltpu.roll(kk, 128 - (d // ROLL) * ROLL, 1))[:, d % ROLL:d % ROLL + 1],
                        (8, TQ))
                    for d in range(DH)]
            return kb_cache[g]

        def vpu_vreg(v, t):
            g, j = v // NQ, v % NQ
            kb = get_kb(g, t)
            if tok(t - LEAD2) is not None:
                kb = [jnp.where(never, tok(t - LEAD2), kb[a]) for a in range(NGATE)] + kb[NGATE:]
            qc, qo = (j * TQ) // CH, (j * TQ) % CH
            accs = [None] * NACC
            for d in range(DH):
                pr = kb[d] * qf_scr[qc, h_qk, d:d + 1, qo:qo + TQ]
                accs[d % NACC] = pr if accs[d % NACC] is None else accs[d % NACC] + pr
            sv = accs[0]
            for a in accs[1:]:
                sv = sv + a
            sv_scr[par_w, j, 8 * g:8 * g + 8, :] = sv
            pending.setdefault(t + LAG, []).append(sv)

        v = 0
        ps = {}
        accs_pv = {}

        def do_pv(tp, t):
            jp, ip = tp // NKT, tp % NKT
            d = lax.dot_general(vt_load(h_pv, ip), ps.pop((jp, ip)), NN, preferred_element_type=F32)
            accs_pv[jp] = d if ip == 0 else accs_pv[jp] + d
            toks[t] = accs_pv[jp][0:8]
            if ip == NKT - 1:
                qo = (jp * TQ) % CH
                ot_scr[(jp * TQ) // CH, h_pv, :, qo:qo + TQ] = accs_pv.pop(jp)

        for j in range(NQ):
            qc, qo = (j * TQ) // CH, (j * TQ) % CH
            band = qb_scr[qc, h_qk, :, qo:qo + TQ]
            groups = [band[0:8], band[8:16]]
            m_new = None
            nps = 0
            if h_pv is not None:
                m_cur = m_final(par_r, j)
            k0 = NV
            for u in range(NKT):
                t = j * NKT + u
                n = sizes[u]
                if h_pv is not None:
                    while nps < max(u + 1, (k0 + n + 127) // 128):
                        ps[(j, nps)] = jnp.exp2(s_tile(par_r, j, nps) - m_cur)
                        nps += 1
                gl = list(groups)
                for a, sv in enumerate(pending.pop(t, [])):
                    gl[1 - a % 2] = jnp.where(never, pltpu.bitcast(sv, U32), gl[1 - a % 2])
                qm = pltpu.bitcast(jnp.concatenate(gl, axis=0), BF16)
                s = jnp.dot(kload(h_qk, k0, n)[:, 0:32], qm, preferred_element_type=F32)
                s_scr[j, k0 - NV:k0 + n - NV, :] = s
                mc = jnp.max(s.reshape(n // 8, 8, TQ), axis=0)
                m_new = mc if m_new is None else jnp.maximum(m_new, mc)
                toks[t] = m_new if TOKM else mc
                k0 += n
                if h_pv is not None and t >= PVLAG:
                    do_pv(t - PVLAG, t)
                while v < NVV and vslot[v] <= t:
                    vpu_vreg(v, t)
                    v += 1
            assert k0 == S
            mm_scr[j] = m_new
        if h_pv is not None:
            for tp in range(NSLOT - PVLAG, NSLOT):
                do_pv(tp, NSLOT - 1)
        assert v == NVV

    stage(None, 0, P_FIRST)

    def body(h, carry):
        stage(h, h + 1, P_MAIN)
        return carry
    lax.fori_loop(0, H - 1, body, 0)
    cp_w1.wait(); cp_w2.wait(); cp_wo.wait(); cp_gw.wait()

    gw = gw_ref[...].astype(F32).reshape(1, D)

    def final(c, carry):
        hs = []
        for jj in range(QPC):
            j = c * QPC + jj
            hs.append(jnp.maximum(
                jnp.dot(x_v[rows_of(j, TQ), :], w1_v[...], preferred_element_type=F32), 0.0).astype(BF16))
            m_cur = m_final((H - 1) % 2, j)
            acc = None
            for i in range(NKT):
                p = jnp.exp2(s_tile((H - 1) % 2, j, i) - m_cur)
                d = lax.dot_general(vt_load(H - 1, i), p, NN, preferred_element_type=F32)
                acc = d if acc is None else acc + d
            ot_scr[c, H - 1, :, jj * TQ:(jj + 1) * TQ] = acc
        hdn = jnp.concatenate(hs, axis=0)
        bb = jnp.dot(hdn, w2_v[...], preferred_element_type=F32)
        ot = jnp.concatenate(
            [ot_scr[c, h, 0:DH, :] * (1.0 / ot_scr[c, h, DH:DH + 1, :]) for h in range(H)], axis=0)
        o = ot.T.astype(BF16)
        for q in range(OSPLIT):
            i = c * OSPLIT + q
            a = jnp.dot(o[q * OR:(q + 1) * OR, :], wo_v[...], preferred_element_type=F32)
            xq = x_v[rows_of(i, OR), :]
            gl = jnp.sum(xq.astype(F32) * gw, axis=-1, keepdims=True)
            g = jax.nn.sigmoid(gl)
            out_v[rows_of(i, OR), :] = (g * a + (1.0 - g) * bb[q * OR:(q + 1) * OR, :]).astype(BF16)
            cp_out(i).start()
        return carry
    lax.fori_loop(0, NC, final, 0)
    for i in range(NO):
        cp_out(i).wait()


@jax.jit
def pallas_gated_mix__softmax_full_mha__dense_activation_relu__prompt_kernel(
    A_x: jax.Array,
    A_wqkv: jax.Array,
    A_wo: jax.Array,
    B_x: jax.Array,
    B_w1: jax.Array,
    B_w2: jax.Array,
    gate_w: jax.Array,
):
    del B_x
    anyspec = pl.BlockSpec(memory_space=pl.ANY)
    out = pl.pallas_call(
        _kernel,
        in_specs=[anyspec] * 6,
        out_specs=anyspec,
        out_shape=jax.ShapeDtypeStruct((S, D), BF16),
        scratch_shapes=[
            pltpu.VMEM((S, D), BF16),
            pltpu.VMEM((3, D, D), BF16),
            pltpu.VMEM((D, D), BF16),
            pltpu.VMEM((D, DFF), BF16),
            pltpu.VMEM((DFF, D), BF16),
            pltpu.VMEM((S, D), BF16),
            pltpu.VMEM((5, S // 2, 128), U32),
            pltpu.VMEM((H, S // 2, 128), U32),
            pltpu.VMEM((NC, H, 24, CH), F32),
            pltpu.VMEM((NC, H, 16, CH), U32),
            pltpu.VMEM((NC, H, 24, CH), F32),
            pltpu.VMEM((3 * D, D), BF16),
            pltpu.VMEM((NQ, S - NV, TQ), F32),
            pltpu.VMEM((2, NQ, NV, TQ), F32),
            pltpu.VMEM((NQ, 8, TQ), F32),
            pltpu.VMEM((NC, H, 24, CH), F32),
            pltpu.VMEM((D,), BF16),
            pltpu.SMEM((1,), jnp.int32),
            pltpu.SemaphoreType.DMA((NC + 9 + NO,)),
        ],
        compiler_params=pltpu.CompilerParams(vmem_limit_bytes=110 * 1024 * 1024),
    )(A_x.reshape(S, D), A_wqkv, A_wo, B_w1, B_w2, gate_w)
    return out.reshape(1, S, D)
```
